```python
import jax
import jax.numpy as jnp

def _softmax(x, axis=-1):
    return jax.nn.softmax(x, axis=axis)

def _gelu(x):
    return jax.nn.gelu(x, approximate=True)

def _silu(x):
    return jax.nn.silu(x)

def _sigmoid(x):
    return jax.nn.sigmoid(x)

def _layernorm(x, axis=-1, eps=1e-05):
    m = jnp.mean(x, axis=axis, keepdims=True)
    v = jnp.var(x, axis=axis, keepdims=True)
    return (x - m) / jnp.sqrt(v + eps)

def _scatter_add(tgt, idx, src, axis=0):
    return tgt.at[idx].add(src)

def _segment_sum(src, seg, n):
    return jax.ops.segment_sum(src, seg, n)

class _Rng:

    def __init__(self, key):
        self._k = key

    def _next(self):
        self._k, sub = jax.random.split(self._k)
        return sub

    def normal(self, shape):
        return jax.random.normal(self._next(), shape, dtype=jnp.bfloat16)

    def randint(self, lo, hi, shape):
        return jax.random.randint(self._next(), shape, lo, hi, dtype=jnp.int32)

    def uniform(self, shape, lo=0.0, hi=1.0):
        return jax.random.uniform(self._next(), shape, jnp.bfloat16, lo, hi)

    def permutation(self, n):
        return jax.random.permutation(self._next(), n)
kernel_name = 'adaLN_cond__compressed_kv_cla__dense_activation_relu__prompt'

def _fwd_setup_inputs():
    _rng = _Rng(jax.random.key(int.from_bytes(__import__("os").urandom(4), "little")))
    _w = lambda a: (lambda t: t.astype(jnp.bfloat16) if jnp.issubdtype(t.dtype, jnp.floating) else t)(jnp.asarray(a))

    def _A_setup():
        B, H, Sq, Sk, D, M = (1, 32, 2048, 2048, 128, 512)
        Dc = 4 * D
        return {'x': _w((lambda *s: _rng.normal(s) * 0.05)(B, Sq, M)), 'c_kv': _w((lambda *s: _rng.normal(s) * 0.05)(B, Sk, Dc)), 'w_q': _w((lambda *s: _rng.normal(s) * 0.05)(M, H, D) * M ** (-0.5)), 'w_uk': _w((lambda *s: _rng.normal(s) * 0.05)(Dc, H, D) * Dc ** (-0.5)), 'w_uv': _w((lambda *s: _rng.normal(s) * 0.05)(Dc, H, D) * Dc ** (-0.5)), 'w_o': _w((lambda *s: _rng.normal(s) * 0.05)(H, D, M) * (H * D) ** (-0.5))}
    _A_in = _A_setup()

    def _B_setup():
        B, S, D, Dff = (1, 2048, 512, 1792)
        return {'x': _w((lambda *s: _rng.normal(s) * 0.05)(B, S, D)), 'w1': _w((lambda *s: _rng.normal(s) * 0.05)(D, Dff)), 'w2': _w((lambda *s: _rng.normal(s) * 0.05)(Dff, D))}
    _B_in = _B_setup()
    return {'A_x': _A_in['x'], 'A_c_kv': _A_in['c_kv'], 'A_w_q': _A_in['w_q'], 'A_w_uk': _A_in['w_uk'], 'A_w_uv': _A_in['w_uv'], 'A_w_o': _A_in['w_o'], 'B_x': _B_in['x'], 'B_w1': _B_in['w1'], 'B_w2': _B_in['w2'], 'c': _w((lambda *s: _rng.normal(s) * 0.05)(1, 512)), 'w_mod': _w((lambda *s: _rng.normal(s) * 0.05)(512, 6 * 512) * 512 ** (-0.5))}

def _fwd_reference(A_x, A_c_kv, A_w_q, A_w_uk, A_w_uv, A_w_o, B_x, B_w1, B_w2, c, w_mod):

    def _A_ref(x, c_kv, w_q, w_uk, w_uv, w_o):
        B, Sq, M = (x.shape[0], x.shape[1], x.shape[2])
        Sk = c_kv.shape[1]
        H, D = (w_q.shape[1], w_q.shape[2])
        q = jnp.einsum('bqm,mhd->bhqd', x, w_q)
        k = jnp.einsum('bkc,chd->bhkd', c_kv, w_uk)
        v = jnp.einsum('bkc,chd->bhkd', c_kv, w_uv)
        scores = jnp.einsum('bhqd,bhkd->bhqk', q, k) * D ** (-0.5)
        off = Sk - Sq
        qi = jnp.arange(Sq)[:, None]
        kj = jnp.arange(Sk)[None, :]
        cmask = kj <= qi + off
        scores = jnp.where(cmask[None, None], scores, -1000000000.0)
        p = _softmax(scores, axis=-1)
        ctx = jnp.einsum('bhqk,bhkd->bhqd', p, v)
        return jnp.einsum('bhqd,hdm->bqm', ctx, w_o)

    def _B_ref(x, w1, w2):
        h = jnp.einsum('bsd,df->bsf', x, w1)
        zero = jnp.zeros_like(h)
        h = jnp.maximum(h, zero)
        return jnp.einsum('bsf,fd->bsd', h, w2)
    x = A_x
    mod = (_silu(c) @ w_mod).reshape(c.shape[0], 6, 1, -1)
    sa, ca, ga, sb, cb, gb = (mod[:, 0].copy(), mod[:, 1].copy(), mod[:, 2].copy(), mod[:, 3].copy(), mod[:, 4].copy(), mod[:, 5].copy())
    h = _layernorm(x, axis=-1) * (1 + ca) + sa
    x = x + ga * _A_ref(h, A_c_kv, A_w_q, A_w_uk, A_w_uv, A_w_o)
    h = _layernorm(x, axis=-1) * (1 + cb) + sb
    x = x + gb * _B_ref(h, B_w1, B_w2)
    return x

def setup_inputs():
    _inp = _fwd_setup_inputs()
    _gk = jax.random.fold_in(jax.random.key(int.from_bytes(__import__("os").urandom(4), "little")), 2 ** 31 - 1)
    _shapes = [[1, 2048, 512]]
    _dtypes = ['bfloat16']
    _gks = jax.random.split(_gk, len(_shapes))
    _gs = [jax.random.normal(k, s, dtype=jnp.dtype(d)) * 0.05 for k, s, d in zip(_gks, _shapes, _dtypes)]
    _inp['grad_out'] = _gs[0]
    return _inp

def reference(A_x, A_c_kv, A_w_q, A_w_uk, A_w_uv, A_w_o, B_w1, B_w2, c, w_mod, B_x, grad_out):
    _const = dict(B_x=B_x)

    def _f(*_d):
        return _fwd_reference(**{'A_x': _d[0], 'A_c_kv': _d[1], 'A_w_q': _d[2], 'A_w_uk': _d[3], 'A_w_uv': _d[4], 'A_w_o': _d[5], 'B_w1': _d[6], 'B_w2': _d[7], 'c': _d[8], 'w_mod': _d[9], **_const})
    _out, _vjp = jax.vjp(_f, A_x, A_c_kv, A_w_q, A_w_uk, A_w_uv, A_w_o, B_w1, B_w2, c, w_mod)
    _grads = _vjp(grad_out)
    _out0 = jnp.asarray(_out)
    return (_out0, *[jnp.asarray(_g) for _g in _grads])
```

```python
import jax
import jax.numpy as jnp
from jax.experimental import pallas as pl
from jax.experimental.pallas import tpu as pltpu

S, M, H, D, C, F = 2048, 512, 32, 128, 512, 1792
G = 8
NG = H // G
B = 128
NB = S // B
RB = 256
NRB = S // RB
FB = 128
NFB = S // FB
EPS = 1e-5
SCALE = D ** -0.5
LOG2E = 1.4426950408889634
LN2 = 0.6931471805599453
MASKED = -1e30
T = NB * (NB + 1) // 2
HP = H - 2
HB = 3
HT = 4
CH = M // G

assert NRB * CH == M and NRB * HB + 2 * HT == H and G == 8 and NB == 16 and T % 2 == 0

BF = jnp.bfloat16
F32 = jnp.float32
NN = (((1,), (0,)), ((), ()))
NT = (((1,), (1,)), ((), ()))


def _dot(a, b, dims=NN):
    return jax.lax.dot_general(a, b, dims, preferred_element_type=F32)


def _causal(st):
    r = jax.lax.broadcasted_iota(jnp.int32, st.shape, 0)
    c = jax.lax.broadcasted_iota(jnp.int32, st.shape, 1)
    return jnp.where(r <= c, st, MASKED)


def _rows(i, n):
    return pl.ds(pl.multiple_of(i * n, n), n)


def _branch(pred, fn):
    def body(_, carry):
        fn()
        return carry
    jax.lax.fori_loop(0, pred.astype(jnp.int32), body, 0)


def _split_rows(v):
    hi = v.astype(BF).astype(F32)
    lo = v - hi
    row = jax.lax.broadcasted_iota(jnp.int32, (16, v.shape[1]), 0)
    return jnp.where(row == 0, hi, jnp.where(row == 1, lo, 0.0)).astype(BF)


def _norm(x):
    mu = jnp.mean(x, axis=1, keepdims=True)
    xc = x - mu
    var = jnp.mean(xc * xc, axis=1, keepdims=True)
    rstd = jax.lax.rsqrt(var + EPS)
    return xc * rstd, rstd


def _norm_bwd(dxh, xh, rstd):
    a = jnp.mean(dxh, axis=1, keepdims=True)
    b = jnp.mean(dxh * xh, axis=1, keepdims=True)
    return rstd * (dxh - a - xh * b)


def _tile(i, j):
    return i * (i + 1) // 2 + j


def _p_tile(p_ref, t):
    return p_ref[t // 2, :, (t % 2) * B:(t % 2 + 1) * B]


def _attn_fwd(k_ref, q_ref, vt_ref, ct_ref, c_ref, p_ref, mrow, la=3, lag=1):
    bl = [(i, j) for i in range(NB) for j in range(i + 1)]

    def scores(b):
        i, j = bl[b]
        st = _dot(k_ref[j * B:(j + 1) * B, :], q_ref[i * B:(i + 1) * B, :], NT)
        return _causal(st) if i == j else st

    acc = {}
    late = []

    def factors(i, lse):
        t0 = _tile(i, 0)
        c_ref[t0:t0 + i + 1, :] = jnp.exp2(mrow[i % 2, 0:i + 1, :] - lse)

    def pv(b, p, alpha, l, m):
        i, j = bl[b]
        o = _dot(vt_ref[:, j * B:(j + 1) * B], p)
        acc[i] = o if j == 0 else alpha * acc[i] + o
        while late:
            factors(*late.pop(0))
        if j == i:
            ct_ref[:, i * B:(i + 1) * B] = (acc.pop(i) * (1.0 / l)).astype(BF)
            late.append((i, m + jnp.log2(l)))

    sts = {b: scores(b) for b in range(la)}
    pend, held = [], []
    m = l = None
    for b in range(len(bl)):
        if b + la < len(bl):
            sts[b + la] = scores(b + la)
        i, j = bl[b]
        st = sts.pop(b)
        mb = jnp.max(st, axis=0, keepdims=True)
        if j == 0:
            m, alpha = mb, None
            p = jnp.exp2(st - m)
            l = jnp.sum(p, axis=0, keepdims=True)
        else:
            m_new = jnp.maximum(m, mb)
            alpha = jnp.exp2(m - m_new)
            m = m_new
            p = jnp.exp2(st - m)
            l = alpha * l + jnp.sum(p, axis=0, keepdims=True)
        mrow[i % 2, j:j + 1, :] = m
        held.append(p)
        if len(held) == 2:
            p_ref[b // 2] = jnp.concatenate(held, axis=1).astype(BF)
            held = []
        pend.append((b, p.astype(BF), alpha, l, m))
        if len(pend) > lag:
            pv(*pend.pop(0))
    while pend:
        pv(*pend.pop(0))
    while late:
        factors(*late.pop(0))


def _attn_bwd(p_ref, c_ref, kt_ref, v_ref, q_ref, dot_ref, dl_ref, dq_ref, dkv_ref, la=2, lag=1):
    bl = [(j, i) for j in range(NB) for i in range(j, NB)]

    def first(b):
        j, i = bl[b]
        return _dot(v_ref[j * B:(j + 1) * B, :], dot_ref[:, i * B:(i + 1) * B])

    def second(b, dpt):
        j, i = bl[b]
        t = _tile(i, j)
        p = _p_tile(p_ref, t).astype(F32) * c_ref[t:t + 1, :]
        ds = p * (dpt - dl_ref[i:i + 1, :])
        return p.astype(BF), ds.astype(BF)

    acc = {}

    def third(b, p, ds):
        j, i = bl[b]
        dv = _dot(p, dot_ref[:, i * B:(i + 1) * B], NT)
        dk = _dot(ds, q_ref[i * B:(i + 1) * B, :])
        dq = _dot(kt_ref[:, j * B:(j + 1) * B], ds)
        if i == j:
            acc['v'], acc['k'] = dv, dk
        else:
            acc['v'], acc['k'] = acc['v'] + dv, acc['k'] + dk
        if j == 0:
            dq_ref[:, i * B:(i + 1) * B] = dq
        else:
            dq_ref[:, i * B:(i + 1) * B] += dq
        if i == NB - 1:
            dkv_ref[j * B:(j + 1) * B, 0:D] = (acc['k'] * LN2).astype(BF)
            dkv_ref[j * B:(j + 1) * B, D:2 * D] = acc['v'].astype(BF)

    s1 = {b: first(b) for b in range(la)}
    pend = []
    for b in range(len(bl)):
        if b + la < len(bl):
            s1[b + la] = first(b + la)
        pend.append((b, *second(b, s1.pop(b))))
        if len(pend) > lag:
            third(*pend.pop(0))
    while pend:
        third(*pend.pop(0))


(SEM_X, SEM_CKV, SEM_WMA, SEM_WMB, SEM_W1, SEM_W2, SEM_G, SEM_S0, SEM_S1, SEM_S2, SEM_WO0, SEM_WO1,
 SEM_OUT0, SEM_OUT1, SEM_DW1, SEM_DW2, SEM_DWO0, SEM_DWO1, SEM_DX, SEM_DC0, SEM_DC1,
 SEM_PO0, SEM_PO1, SEM_PI0, SEM_PI1, SEM_CH) = range(26)
NSEM = SEM_CH + 6


def _silu_parts(c_ref):
    c = c_ref[...].astype(F32)
    sig = jax.nn.sigmoid(c)
    return c, sig


def _outer_cols(dst, c_ref, dmod_v, rows):
    c, sig = _silu_parts(c_ref)
    col = jnp.broadcast_to(c * sig, (B, M)).T
    for n, t in enumerate(rows):
        row = dmod_v[t:t + 1, :]
        for u in range(M // B):
            dst[:, n * M + u * B:n * M + (u + 1) * B] = (col * row[:, u * B:(u + 1) * B]).astype(BF)


def _dsilu_part(wm, dmod_v, rows):
    tot = jnp.zeros((1, M), F32)
    for n, t in enumerate(rows):
        d2 = _dot(_split_rows(dmod_v[t:t + 1, :]), wm[:, n * M:(n + 1) * M], NT)
        tot = tot + d2[0:1] + d2[1:2]
    return tot


def _kernel(c_ref, x_hbm, ckv_hbm, wq_hbm, wk_hbm, wv_hbm, wo_hbm, w1_hbm, w2_hbm, wmod_hbm, g_hbm,
            out_hbm, dx_hbm, dckv_hbm, dwq_hbm, dwk_hbm, dwv_hbm, dwo_hbm, dw1_hbm, dw2_hbm,
            dc_ref, dwmod_hbm, p_hbm,
            q_all, kt_all, v_all, ct_all, c_all, pbuf, wq_hm, wk_hm, wv_hm, hct, acc_a, dattn, dx1,
            x_v, wo_buf, mod_v, dmod_v, w1_v, w2_v, wm_b, st_q, st_k, st_v, sems):
    cp = pltpu.make_async_copy
    w_hbm = (wq_hbm, wk_hbm, wv_hbm)
    dw_hbm = (dwq_hbm, dwk_hbm, dwv_hbm)
    w_hm = (wq_hm, wk_hm, wv_hm)
    st = (st_q, st_k, st_v)

    def wo_copy(h, slot):
        return cp(wo_hbm.at[h], wo_buf.at[slot], sems.at[SEM_WO0 + slot])

    def p_out(h, slot):
        return cp(pbuf.at[slot], p_hbm.at[h], sems.at[SEM_PO0 + slot])

    def p_in(h, slot):
        return cp(p_hbm.at[h], pbuf.at[slot], sems.at[SEM_PI0 + slot])

    def mod_rows(wm, first, n):
        c, sig = _silu_parts(c_ref)
        mod2 = _dot(_split_rows(c * sig), wm[...])
        mod = mod2[0:1] + mod2[1:2]
        for t in range(n):
            mod_v[first + t:first + t + 1, :] = mod[:, t * M:(t + 1) * M]

    x_copy = cp(x_hbm, x_v, sems.at[SEM_X])
    w1_copy = cp(w1_hbm, w1_v, sems.at[SEM_W1])
    w2_copy = cp(w2_hbm, w2_v, sems.at[SEM_W2])
    g_copy = cp(g_hbm, dattn, sems.at[SEM_G])
    dw1_copy = cp(w1_v, dw1_hbm, sems.at[SEM_DW1])
    dw2_copy = cp(w2_v, dw2_hbm, sems.at[SEM_DW2])
    wmb_copy = cp(wmod_hbm.at[:, pl.ds(2 * M, 4 * M)], wm_b, sems.at[SEM_WMB])
    dwmb_copy = cp(wm_b, dwmod_hbm.at[:, pl.ds(2 * M, 4 * M)], sems.at[SEM_WMB])

    def fwd_and_ffn():
        def fwd(hc, vt, k_v, mrow):
            def chunk_in(t):
                gs = pl.ds(pl.multiple_of((((t >> 3) + 1) & (NG - 1)) * G, G), G)
                rows = _rows(t & (G - 1), CH)
                return [cp(w_hbm[n].at[rows, gs, :], st[n].at[t & 1], sems.at[SEM_CH + 3 * (t & 1) + n])
                        for n in range(3)]

            ckv_copy = cp(ckv_hbm, hc.at[1], sems.at[SEM_CKV])

            def prologue(wm_a, s0, s1, s2):
                big = (s0, s1, s2)
                wma_copy = cp(wmod_hbm.at[:, pl.ds(0, 2 * M)], wm_a, sems.at[SEM_WMA])
                big_in = [cp(w_hbm[n].at[:, pl.ds(0, G), :], big[n], sems.at[SEM_S0 + n])
                          for n in range(3)]
                wma_copy.start()
                x_copy.start()
                for n in range(3):
                    big_in[n].start()
                ckv_copy.start()
                acc_a[...] = jnp.zeros(acc_a.shape, F32)
                wma_copy.wait()
                mod_rows(wm_a, 0, 2)
                x_copy.wait()

                for r in range(NRB):
                    rows = slice(r * RB, (r + 1) * RB)
                    xh, _ = _norm(x_v[rows, :].astype(F32))
                    hc[0, rows, :] = (xh * (1.0 + mod_v[1:2, :]) + mod_v[0:1, :]).astype(BF)
                for n in range(3):
                    big_in[n].wait()
                    for cc in range(G):
                        w_hm[n][0:G, cc * CH:(cc + 1) * CH, :] = jnp.swapaxes(
                            big[n][cc * CH:(cc + 1) * CH], 0, 1)
                wo_copy(0, 0).start()
                for cc in chunk_in(0):
                    cc.start()
                ckv_copy.wait()
                wmb_copy.start()
                w1_copy.start()
                w2_copy.start()
                g_copy.start()

            pl.run_scoped(prologue, pltpu.VMEM((M, 2 * M), BF), pltpu.VMEM((M, G, D), BF),
                          pltpu.VMEM((C, G, D), BF), pltpu.VMEM((C, G, D), BF))

            def head(h, carry):
                slot = h & 1
                wo_copy(h, slot).wait()
                wo_copy(jnp.where(h + 1 < H, h + 1, H - 2), 1 - slot).start()
                for cc in chunk_in(h):
                    cc.wait()

                @pl.when(h + 1 < H)
                def _():
                    for cc in chunk_in(h + 1):
                        cc.start()

                @pl.when(h >= 2)
                def _():
                    p_out(h - 2, slot).wait()

                q_all[h] = (_dot(hc[0], wq_hm[h]) * (SCALE * LOG2E)).astype(BF)
                kv = _dot(hc[1], jnp.concatenate([wk_hm[h], wv_hm[h]], axis=1))
                kb = kv[:, :D].astype(BF)
                k_v[...] = kb
                kt_all[h] = kb.T
                vb = kv[:, D:].astype(BF)
                v_all[h] = vb
                vt[...] = vb.T
                gs = pl.ds(pl.multiple_of((((h >> 3) + 1) & (NG - 1)) * G, G), G)
                for n in range(3):
                    w_hm[n][gs, _rows(h & (G - 1), CH), :] = jnp.swapaxes(st[n][slot], 0, 1)
                tr = _rows(h & (NB - 1), B)
                hct[h >> 4, :, tr] = hc[h >> 4, tr, :].T
                _attn_fwd(k_v, q_all.at[h], vt, ct_all.at[h], c_all.at[h], pbuf.at[slot], mrow)
                acc_a[...] += _dot(wo_buf[slot].T, ct_all[h])

                @pl.when(h < HP)
                def _():
                    p_out(h, slot).start()

                return carry

            jax.lax.fori_loop(0, H, head, 0)

        pl.run_scoped(fwd, pltpu.VMEM((2, S, M), BF), pltpu.VMEM((D, S), BF), pltpu.VMEM((S, D), BF),
                      pltpu.VMEM((2, NB, B), F32))

        def ffn(dw1_acc, dw2t_acc, out_st, x1_s, attn_s, h2_s):
            def out_copy(r, slot):
                return cp(out_st.at[slot], out_hbm.at[_rows(r, FB), :], sems.at[SEM_OUT0 + slot])

            dmod_v[...] = jnp.zeros(dmod_v.shape, F32)
            wmb_copy.wait()
            mod_rows(wm_b, 2, 4)

            def front(r):
                rows = _rows(r, FB)
                attn = acc_a[:, rows].T
                x1 = x_v[rows, :].astype(F32) + mod_v[2:3, :] * attn
                xh, _ = _norm(x1)
                attn_s[r & 1] = attn
                x1_s[r & 1] = x1
                h2_s[r & 1] = (xh * (1.0 + mod_v[4:5, :]) + mod_v[3:4, :]).astype(BF)

            front(0)
            w1_copy.wait()
            w2_copy.wait()
            g_copy.wait()

            def block(r, carry):
                rows = _rows(r, FB)
                slot = r & 1

                @pl.when(r >= 2)
                def _():
                    out_copy(r - 2, slot).wait()

                ga, cb, gb = (mod_v[t:t + 1, :] for t in (2, 4, 5))
                h2 = h2_s[slot]
                u = _dot(h2, w1_v[...])
                front(jnp.minimum(r + 1, NFB - 1))
                acc_a[:, rows] = jnp.zeros((M, FB), F32)
                rl = jnp.maximum(u, 0.0).astype(BF)
                f = _dot(rl, w2_v[...])
                x1 = x1_s[slot]
                out_st[slot] = (x1 + gb * f).astype(BF)
                out_copy(r, slot).start()
                g = dattn[rows, :].astype(F32)
                df = (g * gb).astype(BF)
                dr = _dot(df, w2_v[...], NT)
                du = jnp.where(u > 0.0, dr, jnp.where(u == 0.0, 0.5 * dr, 0.0)).astype(BF)
                dh2 = _dot(du, w1_v[...], NT)
                dw2t_acc[...] = jnp.where(r == 0, 0.0, dw2t_acc[...]) + _dot(df.T, rl)
                dw1_acc[...] = jnp.where(r == 0, 0.0, dw1_acc[...]) + _dot(h2.T, du)
                xh, rstd = _norm(x1)
                d1 = g + _norm_bwd(dh2 * (1.0 + cb), xh, rstd)
                dx1[rows, :] = d1
                dattn[rows, :] = (d1 * ga).astype(BF)
                dmod_v[2:3, :] += jnp.sum(d1 * attn_s[slot], axis=0, keepdims=True)
                dmod_v[3:4, :] += jnp.sum(dh2, axis=0, keepdims=True)
                dmod_v[4:5, :] += jnp.sum(dh2 * xh, axis=0, keepdims=True)
                dmod_v[5:6, :] += jnp.sum(g * f, axis=0, keepdims=True)
                return carry

            jax.lax.fori_loop(0, NFB, block, 0)
            dmod_v[6:7, :] = _dsilu_part(wm_b, dmod_v, (2, 3, 4, 5))
            _outer_cols(wm_b, c_ref, dmod_v, (2, 3, 4, 5))
            dwmb_copy.start()
            w1_v[...] = dw1_acc[...].astype(BF)
            dw1_copy.start()
            for t in range(F // 256):
                w2_v[t * 256:(t + 1) * 256, :] = dw2t_acc[:, t * 256:(t + 1) * 256].T.astype(BF)
            dw2_copy.start()
            out_copy(NFB - 2, 0).wait()
            out_copy(NFB - 1, 1).wait()

        pl.run_scoped(ffn, pltpu.VMEM((M, F), F32), pltpu.VMEM((M, F), F32),
                      pltpu.VMEM((2, FB, M), BF), pltpu.VMEM((2, FB, M), F32),
                      pltpu.VMEM((2, FB, M), F32), pltpu.VMEM((2, FB, M), BF))

    fwd_and_ffn()

    def bwd(acc_c):
        def heads(dot_s, dl, dq_acc, dkv):
            def head(t, carry):
                h = H - 1 - t
                slot = h & 1

                @pl.when(t >= 1)
                def _():
                    wo_copy(h, slot).wait()

                @pl.when(jnp.logical_and(t >= 1, h >= 1))
                def _():
                    wo_copy(h - 1, 1 - slot).start()

                @pl.when(h < HP)
                def _():
                    p_in(h, slot).wait()

                @pl.when(jnp.logical_and(h <= HP, h >= 1))
                def _():
                    p_in(h - 1, 1 - slot).start()

                dob = _dot(wo_buf[slot], dattn[...], NT).astype(BF)
                dot_s[...] = dob
                delta = jnp.sum(dob.astype(F32) * ct_all[h].astype(F32), axis=0, keepdims=True)
                for i in range(NB):
                    dl[i:i + 1, :] = delta[:, i * B:(i + 1) * B]
                _attn_bwd(pbuf.at[slot], c_all.at[h], kt_all.at[h], v_all.at[h], q_all.at[h], dot_s,
                          dl, dq_acc, dkv)
                dqt = (dq_acc[...] * SCALE).astype(BF)
                acc_a[...] += _dot(wq_hm[h], dqt)
                wq_hm[h] = _dot(hct[0], dqt, NT).astype(BF)
                acc_c[...] = jnp.where(t == 0, 0.0, acc_c[...]) + _dot(
                    dkv[...], jnp.concatenate([wk_hm[h], wv_hm[h]], axis=1), NT)
                dwkv = _dot(hct[1], dkv[...])
                wk_hm[h] = dwkv[:, :D].astype(BF)
                wv_hm[h] = dwkv[:, D:].astype(BF)
                return carry

            jax.lax.fori_loop(0, H, head, 0)

        pl.run_scoped(heads, pltpu.VMEM((D, S), BF), pltpu.VMEM((NB, B), F32),
                      pltpu.VMEM((D, S), F32), pltpu.VMEM((S, 2 * D), BF))

        def epilogue(wm_a, dwo_st, dc_st, dw_st):
            wma_copy = cp(wmod_hbm.at[:, pl.ds(0, 2 * M)], wm_a, sems.at[SEM_WMA])
            wma_copy.start()

            def dx_copy(r):
                return cp(x_v.at[_rows(r, RB), :], dx_hbm.at[_rows(r, RB), :], sems.at[SEM_DX])

            def dc_copy(r, slot):
                return cp(dc_st.at[slot], dckv_hbm.at[_rows(r, RB), :], sems.at[SEM_DC0 + slot])

            def dwo_heads(first, n, slot):
                ct = ct_all[pl.ds(first, n)].reshape(n * D, S)
                dwo_st[slot, 0:n] = _dot(ct, dattn[...]).astype(BF).reshape(n, D, M)

            def dwo_copy(first, n, slot):
                return cp(dwo_st.at[slot, 0:n], dwo_hbm.at[pl.ds(first, n)], sems.at[SEM_DWO0 + slot])

            def dw_copies(r, slot):
                return [cp(dw_st.at[slot, n], dw_hbm[n].at[_rows(r, CH)], sems.at[SEM_CH + 3 * slot + n])
                        for n in range(3)]

            def send(r):
                for cc in dw_copies(r, r & 1):
                    cc.start()
                dc_copy(r, r & 1).start()
                dx_copy(r).start()
                dwo_copy(r * HB, HB, r & 1).start()

            def block(r, carry):
                rows = _rows(r, RB)
                slot = r & 1

                @pl.when(r >= 2)
                def _():
                    for cc in dw_copies(r - 2, slot):
                        cc.wait()
                    dc_copy(r - 2, slot).wait()
                    dwo_copy((r - 2) * HB, HB, slot).wait()

                _branch(r >= 1, lambda: send(r - 1))

                for n in range(3):
                    for g in range(NG):
                        dw_st[slot, n, :, g * G:(g + 1) * G, :] = jnp.swapaxes(
                            w_hm[n][g * G:(g + 1) * G, _rows(r, CH), :], 0, 1)
                dc_st[slot] = acc_c[rows, :].astype(BF)
                dh1 = acc_a[:, rows].T
                xh, rstd = _norm(x_v[rows, :].astype(F32))
                dmod_v[0:1, :] += jnp.sum(dh1, axis=0, keepdims=True)
                dmod_v[1:2, :] += jnp.sum(dh1 * xh, axis=0, keepdims=True)
                d0 = dx1[rows, :] + _norm_bwd(dh1 * (1.0 + mod_v[1:2, :]), xh, rstd)
                x_v[rows, :] = d0.astype(BF)
                dwo_heads(r * HB, HB, slot)
                return carry

            jax.lax.fori_loop(0, NRB, block, 0)
            send(NRB - 1)
            wma_copy.wait()
            dsc = dmod_v[6:7, :] + _dsilu_part(wm_a, dmod_v, (0, 1))
            _outer_cols(wm_a, c_ref, dmod_v, (0, 1))
            dwma_copy = cp(wm_a, dwmod_hbm.at[:, pl.ds(0, 2 * M)], sems.at[SEM_WMA])
            dwma_copy.start()
            c, sig = _silu_parts(c_ref)
            dc_ref[...] = (dsc * (sig * (1.0 + c * (1.0 - sig)))).astype(BF)

            def last_heads(n, carry):
                dwo_copy((NRB - 2 + n) * HB, HB, n).wait()
                dwo_heads(NRB * HB + n * HT, HT, n)
                dwo_copy(NRB * HB + n * HT, HT, n).start()
                return carry

            jax.lax.fori_loop(0, 2, last_heads, 0)
            for r in range(NRB):
                dx_copy(r).wait()
            for r in (NRB - 2, NRB - 1):
                dc_copy(r, r % 2).wait()
                dwo_copy(NRB * HB + (r % 2) * HT, HT, r % 2).wait()
                for cc in dw_copies(r, r % 2):
                    cc.wait()
            dwma_copy.wait()

        pl.run_scoped(epilogue, pltpu.VMEM((M, 2 * M), BF), pltpu.VMEM((2, HT, D, M), BF),
                      pltpu.VMEM((2, RB, C), BF), pltpu.VMEM((2, 3, CH, H, D), BF))

    pl.run_scoped(bwd, pltpu.VMEM((S, C), F32))
    dw1_copy.wait()
    dw2_copy.wait()
    dwmb_copy.wait()


@jax.jit
def pallas_adaLN_cond__compressed_kv_cla__dense_activation_relu__prompt_kernel(
    A_x, A_c_kv, A_w_q, A_w_uk, A_w_uv, A_w_o, B_x, B_w1, B_w2, c, w_mod, grad_out,
):
    del B_x
    sds = jax.ShapeDtypeStruct
    any_spec = pl.BlockSpec(memory_space=pl.ANY)
    vmem_spec = pl.BlockSpec(memory_space=pltpu.VMEM)
    out_shape = (
        sds((S, M), BF), sds((S, M), BF), sds((S, C), BF),
        sds((M, H, D), BF), sds((C, H, D), BF), sds((C, H, D), BF), sds((H, D, M), BF),
        sds((M, F), BF), sds((F, M), BF), sds((1, M), BF), sds((M, 6 * M), BF),
        sds((HP, T // 2, B, 2 * B), BF),
    )
    scratch = [
        pltpu.VMEM((H, S, D), BF), pltpu.VMEM((H, D, S), BF), pltpu.VMEM((H, S, D), BF),
        pltpu.VMEM((H, D, S), BF), pltpu.VMEM((H, T, B), F32), pltpu.VMEM((2, T // 2, B, 2 * B), BF),
        pltpu.VMEM((H, M, D), BF), pltpu.VMEM((H, C, D), BF), pltpu.VMEM((H, C, D), BF),
        pltpu.VMEM((2, M, S), BF), pltpu.VMEM((M, S), F32),
        pltpu.VMEM((S, M), BF), pltpu.VMEM((S, M), F32),
        pltpu.VMEM((S, M), BF), pltpu.VMEM((2, D, M), BF),
        pltpu.VMEM((8, M), F32), pltpu.VMEM((8, M), F32),
        pltpu.VMEM((M, F), BF), pltpu.VMEM((F, M), BF), pltpu.VMEM((M, 4 * M), BF),
        pltpu.VMEM((2, CH, G, D), BF), pltpu.VMEM((2, CH, G, D), BF), pltpu.VMEM((2, CH, G, D), BF),
        pltpu.SemaphoreType.DMA((NSEM,)),
    ]
    outs = pl.pallas_call(
        _kernel,
        out_shape=out_shape,
        in_specs=[vmem_spec] + [any_spec] * 10,
        out_specs=(any_spec,) * 9 + (vmem_spec, any_spec, any_spec),
        scratch_shapes=scratch,
        compiler_params=pltpu.CompilerParams(vmem_limit_bytes=127 * 1024 * 1024,
                                             disable_bounds_checks=True),
        name="adaln_mla_ffn_fwd_bwd",
    )(c, A_x.reshape(S, M), A_c_kv.reshape(S, C), A_w_q, A_w_uk, A_w_uv, A_w_o, B_w1, B_w2, w_mod,
      grad_out.reshape(S, M))
    out, dx, dckv = (o.reshape(1, S, M) for o in outs[:3])
    return (out, dx, dckv) + tuple(outs[3:11])
```
